```python
import os as _os
_os.environ.setdefault('JAX_PLATFORMS', 'cpu')
import jax
import jax.numpy as jnp

def _softmax(x, axis=-1):
    return jax.nn.softmax(x, axis=axis)

def _gelu(x):
    return jax.nn.gelu(x, approximate=True)

def _silu(x):
    return jax.nn.silu(x)

def _sigmoid(x):
    return jax.nn.sigmoid(x)

def _layernorm(x, axis=-1, eps=1e-05):
    m = jnp.mean(x, axis=axis, keepdims=True)
    v = jnp.var(x, axis=axis, keepdims=True)
    return (x - m) / jnp.sqrt(v + eps)

def _scatter_add(tgt, idx, src, axis=0):
    return tgt.at[idx].add(src)

def _segment_sum(src, seg, n):
    return jax.ops.segment_sum(src, seg, n)

class _Rng:

    def __init__(self, key):
        self._k = key

    def _next(self):
        self._k, sub = jax.random.split(self._k)
        return sub

    def normal(self, shape):
        return jax.random.normal(self._next(), shape, dtype=jnp.bfloat16)

    def randint(self, lo, hi, shape):
        return jax.random.randint(self._next(), shape, lo, hi, dtype=jnp.int32)

    def uniform(self, shape, lo=0.0, hi=1.0):
        return jax.random.uniform(self._next(), shape, jnp.bfloat16, lo, hi)

    def permutation(self, n):
        return jax.random.permutation(self._next(), n)
kernel_name = 'adaLN_cond__mha_block__dense_activation_squared_relu__prompt'

def setup_inputs():
    _rng = _Rng(jax.random.key(int.from_bytes(__import__("os").urandom(4), "little")))
    _w = lambda a: (lambda t: t.astype(jnp.bfloat16) if jnp.issubdtype(t.dtype, jnp.floating) else t)(jnp.asarray(a))

    def _A_setup():
        B, S, D, H = (1, 2048, 512, 32)
        return {'x': _w((lambda *s: _rng.normal(s) * 0.05)(B, S, D)), 'wqkv': _w((lambda *s: _rng.normal(s) * 0.1)(D, 3 * D)), 'wo': _w((lambda *s: _rng.normal(s) * 0.05)(D, D))}
    _A_in = _A_setup()

    def _B_setup():
        B, S, D, F = (1, 2048, 512, 1792)
        return {'x': _w((lambda *s: _rng.normal(s) * 0.05)(B, S, D)), 'w1': _w((lambda *s: _rng.normal(s) * 0.05)(D, F)), 'b1': _w((lambda *s: _rng.normal(s) * 0.05)(F)), 'w2': _w((lambda *s: _rng.normal(s) * 0.05)(F, D)), 'b2': _w((lambda *s: _rng.normal(s) * 0.05)(D))}
    _B_in = _B_setup()
    return {'A_x': _A_in['x'], 'A_wqkv': _A_in['wqkv'], 'A_wo': _A_in['wo'], 'B_x': _B_in['x'], 'B_w1': _B_in['w1'], 'B_b1': _B_in['b1'], 'B_w2': _B_in['w2'], 'B_b2': _B_in['b2'], 'c': _w((lambda *s: _rng.normal(s) * 0.05)(1, 512) * 8.0), 'w_mod': _w((lambda *s: _rng.normal(s) * 0.05)(512, 6 * 512) * 512 ** (-0.5) * 8.0)}

def reference(A_x, A_wqkv, A_wo, B_x, B_w1, B_b1, B_w2, B_b2, c, w_mod):

    def _A_ref(x, wqkv, wo):
        B, S, D = x.shape
        H = 32
        Dh = D // H
        qkv = (lambda x, *d: x.transpose(*d))((x @ wqkv).reshape(B, S, 3, H, Dh), 2, 0, 3, 1, 4)
        q, k, v = (qkv[0], qkv[1], qkv[2])
        scores = jnp.einsum('bhqd,bhkd->bhqk', q, k) * Dh ** (-0.5)
        p = _softmax(scores, axis=-1)
        o = jnp.einsum('bhqk,bhkd->bhqd', p, v)
        return (lambda x, *d: x.transpose(*d))(o, 0, 2, 1, 3).reshape(B, S, D) @ wo

    def _B_ref(x, w1, b1, w2, b2):
        h = jnp.einsum('bsd,df->bsf', x, w1) + b1
        zero = jnp.zeros_like(h)
        r = jnp.where(h > zero, h, zero)
        h = r * r
        out = jnp.einsum('bsf,fd->bsd', h, w2) + b2
        return out
    x = A_x
    mod = (_silu(c) @ w_mod).reshape(c.shape[0], 6, 1, -1)
    sa, ca, ga, sb, cb, gb = (mod[:, 0].copy(), mod[:, 1].copy(), mod[:, 2].copy(), mod[:, 3].copy(), mod[:, 4].copy(), mod[:, 5].copy())
    h = _layernorm(x, axis=-1) * (1 + ca) + sa
    x = x + ga * _A_ref(h, A_wqkv, A_wo)
    h = _layernorm(x, axis=-1) * (1 + cb) + sb
    x = x + gb * _B_ref(h, B_w1, B_b1, B_w2, B_b2)
    return x
```

```python
import functools
import math

import jax
import jax.numpy as jnp
from jax import lax
import jax.experimental.pallas as pl
import jax.experimental.pallas.tpu as pltpu

S = 2048
D = 512
H = 32
DH = 16
F = 1792
TQ = 512
TK = 128
NK = S // TK
EPS = 1e-5
QSCALE = (DH ** -0.5) * math.log2(math.e)

_NT = (((1,), (1,)), ((), ()))


def _ln(x):
    mu = jnp.mean(x, axis=-1, keepdims=True)
    xc = x - mu
    var = jnp.mean(xc * xc, axis=-1, keepdims=True)
    return xc * lax.rsqrt(var + EPS)


def _kernel(x_ref, wqkvT_ref, wk_ref, wo_ref, w1_ref, b1_ref, w2_ref, b2_ref, c_ref, wmod_ref,
            out_ref,
            mod_ref, k_ref, qT_ref, vT_ref, w_ref, sA, sB, mA, mB, oT_ref):
    step = pl.program_id(0)
    f32 = jnp.float32
    bf16 = jnp.bfloat16

    @pl.when(step == 0)
    def _():
        cc = c_ref[...].astype(f32)
        sc = (cc * jax.nn.sigmoid(cc)).astype(bf16)
        mod_ref[...] = jnp.dot(sc, wmod_ref[...], preferred_element_type=f32)
        w_ref[...] = jnp.zeros_like(w_ref)
        sa = mod_ref[0:1, 0 * D:1 * D]
        ca = mod_ref[0:1, 1 * D:2 * D]
        RB = 512
        for r in range(S // RB):
            xr = x_ref[r * RB:(r + 1) * RB, :].astype(f32)
            h = (_ln(xr) * (1.0 + ca) + sa).astype(bf16)
            kk = jnp.dot(h, wk_ref[...], preferred_element_type=f32).astype(bf16)
            for g in range(4):
                k_ref[g, r * RB:(r + 1) * RB, :] = kk[:, g * 128:(g + 1) * 128]
            qT = lax.dot_general(wqkvT_ref[0:D, :], h, _NT, preferred_element_type=f32)
            qT_ref[:, r * RB:(r + 1) * RB] = (qT * QSCALE).astype(bf16)
            vT = lax.dot_general(wqkvT_ref[2 * D:3 * D, :], h, _NT, preferred_element_type=f32)
            vT_ref[:, r * RB:(r + 1) * RB] = vT.astype(bf16)

    q0 = pl.multiple_of(step * TQ, TQ)
    for h in range(H):
        j = h % 8
        w_ref[h, j * 16:(j + 1) * 16, :] = qT_ref[h * 16:(h + 1) * 16, pl.ds(q0, TQ)]

    def fused(h1, s1, m1, h2, s2, m2):
        if h1 is not None:
            g = h1 // 8
            w = w_ref[h1]
            m8 = None
        if h2 is not None:
            m = m2[...]
            l8 = None
            acc = None
        for c in range(NK):
            if h1 is not None:
                sT = jnp.dot(k_ref[g, c * TK:(c + 1) * TK, :], w, preferred_element_type=f32)
                s1[c * TK:(c + 1) * TK, :] = sT
                mc = jnp.max(sT.reshape(TK // 8, 8, TQ), axis=0)
                m8 = mc if m8 is None else jnp.maximum(m8, mc)
            if h2 is not None:
                p = jnp.exp2(s2[c * TK:(c + 1) * TK, :] - m)
                lc = jnp.sum(p.reshape(TK // 8, 8, TQ), axis=0)
                l8 = lc if l8 is None else l8 + lc
                vh = vT_ref[pl.ds(pl.multiple_of(h2 * 16, 16), 16), c * TK:(c + 1) * TK]
                a = jnp.dot(vh, p.astype(bf16), preferred_element_type=f32)
                acc = a if acc is None else acc + a
        if h1 is not None:
            m1[...] = jnp.max(m8, axis=0, keepdims=True)
        if h2 is not None:
            l = jnp.sum(l8, axis=0, keepdims=True)
            oT_ref[pl.ds(pl.multiple_of(h2 * 16, 16), 16), :] = acc / l

    fused(0, sA, mA, None, None, None)

    def body(h, carry):
        @pl.when(h % 2 == 0)
        def _():
            fused(h + 1, sB, mB, h, sA, mA)

        @pl.when(h % 2 == 1)
        def _():
            fused(h + 1, sA, mA, h, sB, mB)
        return carry

    lax.fori_loop(0, H - 1, body, 0)
    fused(None, None, None, H - 1, sB, mB)

    ga = mod_ref[0:1, 2 * D:3 * D]
    sb = mod_ref[0:1, 3 * D:4 * D]
    cb = mod_ref[0:1, 4 * D:5 * D]
    gb = mod_ref[0:1, 5 * D:6 * D]
    o = oT_ref[...].T.astype(bf16)
    attn = jnp.dot(o, wo_ref[...], preferred_element_type=f32)
    x1 = x_ref[pl.ds(q0, TQ), :].astype(f32) + ga * attn
    h2 = (_ln(x1) * (1.0 + cb) + sb).astype(bf16)
    u = jnp.dot(h2, w1_ref[...], preferred_element_type=f32) + b1_ref[...].astype(f32)
    r = jnp.maximum(u, 0.0)
    hh = (r * r).astype(bf16)
    y = jnp.dot(hh, w2_ref[...], preferred_element_type=f32) + b2_ref[...].astype(f32)
    out_ref[...] = (x1 + gb * y).astype(out_ref.dtype)


@jax.jit
def pallas_adaLN_cond__mha_block__dense_activation_squared_relu__prompt_kernel(
    A_x: jax.Array,
    A_wqkv: jax.Array,
    A_wo: jax.Array,
    B_x: jax.Array,
    B_w1: jax.Array,
    B_b1: jax.Array,
    B_w2: jax.Array,
    B_b2: jax.Array,
    c: jax.Array,
    w_mod: jax.Array,
):
    del B_x
    x2 = A_x.reshape(S, D)
    wqkvT = A_wqkv.T
    wk = A_wqkv[:, D:2 * D]
    c8 = jnp.broadcast_to(c, (8, D))
    b1 = B_b1.reshape(1, F)
    b2 = B_b2.reshape(1, D)

    def full(shape):
        return pl.BlockSpec(shape, lambda i: (0,) * len(shape))

    out = pl.pallas_call(
        _kernel,
        grid=(S // TQ,),
        in_specs=[
            full((S, D)), full((3 * D, D)), full((D, D)), full((D, D)), full((D, F)), full((1, F)),
            full((F, D)), full((1, D)), full((8, D)), full((D, 6 * D)),
        ],
        out_specs=pl.BlockSpec((TQ, D), lambda i: (i, 0)),
        out_shape=jax.ShapeDtypeStruct((S, D), A_x.dtype),
        scratch_shapes=[
            pltpu.VMEM((8, 6 * D), jnp.float32),
            pltpu.VMEM((4, S, 128), jnp.bfloat16),
            pltpu.VMEM((D, S), jnp.bfloat16),
            pltpu.VMEM((D, S), jnp.bfloat16),
            pltpu.VMEM((H, 128, TQ), jnp.bfloat16),
            pltpu.VMEM((S, TQ), jnp.float32),
            pltpu.VMEM((S, TQ), jnp.float32),
            pltpu.VMEM((1, TQ), jnp.float32),
            pltpu.VMEM((1, TQ), jnp.float32),
            pltpu.VMEM((D, TQ), jnp.float32),
        ],
        compiler_params=pltpu.CompilerParams(
            dimension_semantics=("arbitrary",),
            vmem_limit_bytes=100 * 1024 * 1024,
        ),
    )(x2, wqkvT, wk, A_wo, B_w1, b1, B_w2, b2, c8, w_mod)
    return out.reshape(A_x.shape)
```

```python
import functools
import math

import jax
import jax.numpy as jnp
from jax import lax
import jax.experimental.pallas as pl
import jax.experimental.pallas.tpu as pltpu

S = 2048
D = 512
H = 32
DH = 16
F = 1792
TQ = 512
TK = 128
NK = S // TK
XB = (0, 256, 2048)
RBS = (0, 256, 384, 768, 1280, 2048)
LAG = 2
FB = 512
EPS = 1e-5
QSCALE = (DH ** -0.5) * math.log2(math.e)

_NT = (((1,), (1,)), ((), ()))


def _ln(x):
    mu = jnp.mean(x, axis=-1, keepdims=True)
    xc = x - mu
    var = jnp.mean(xc * xc, axis=-1, keepdims=True)
    return xc * lax.rsqrt(var + EPS)


def _kernel(x_hbm, wqkv_hbm, wo_hbm, w1_hbm, b1_ref, w2_hbm, b2_ref, c_ref, wmod_hbm,
            out_ref,
            x_ref, wqkv_ref, wo_ref, w1_ref, w2_ref, wmod_ref, sems,
            mod_ref, k_ref, qT_ref, vT_ref, w_ref, s_ref, m_ref, oT_ref):
    step = pl.program_id(0)
    f32 = jnp.float32
    bf16 = jnp.bfloat16

    def cp_wmod_a():
        return pltpu.make_async_copy(wmod_hbm.at[:, 0:2 * D], wmod_ref.at[:, 0:2 * D], sems.at[0])

    def cp_x(r):
        lo, hi = XB[r], XB[r + 1]
        return pltpu.make_async_copy(x_hbm.at[lo:hi, :], x_ref.at[lo:hi, :], sems.at[1 + r])

    def cp_wqkv():
        return pltpu.make_async_copy(wqkv_hbm, wqkv_ref, sems.at[5])

    def cp_wmod_b():
        return pltpu.make_async_copy(wmod_hbm.at[:, 2 * D:6 * D], wmod_ref.at[:, 2 * D:6 * D], sems.at[6])

    def cp_wo():
        return pltpu.make_async_copy(wo_hbm, wo_ref, sems.at[7])

    def cp_w1():
        return pltpu.make_async_copy(w1_hbm, w1_ref, sems.at[8])

    def cp_w2():
        return pltpu.make_async_copy(w2_hbm, w2_ref, sems.at[9])

    def silu_c():
        cc = jnp.broadcast_to(c_ref[...].astype(f32), (8, D))
        return (cc * jax.nn.sigmoid(cc)).astype(bf16)

    @pl.when(step == 0)
    def _():
        cp_wmod_a().start()
        cp_x(0).start()
        cp_wqkv().start()
        cp_x(1).start()

        w_ref[...] = jnp.zeros_like(w_ref)
        cp_wmod_a().wait()
        mod_ref[:, 0:2 * D] = jnp.dot(silu_c(), wmod_ref[:, 0:2 * D], preferred_element_type=f32)
        sa = mod_ref[0:1, 0 * D:1 * D]
        ca = mod_ref[0:1, 1 * D:2 * D]
        cp_wqkv().wait()
        cp_x(0).wait()
        cp_wmod_b().start()
        cp_wo().start()
        cp_w1().start()
        cp_w2().start()
        wqT = wqkv_ref[:, 0:D].T
        wvT = wqkv_ref[:, 2 * D:3 * D].T
        for r in range(len(RBS) - 1):
            lo, hi = RBS[r], RBS[r + 1]
            if lo == XB[1]:
                cp_x(1).wait()
            xr = x_ref[lo:hi, :].astype(f32)
            h = (_ln(xr) * (1.0 + ca) + sa).astype(bf16)
            kk = jnp.dot(h, wqkv_ref[:, D:2 * D], preferred_element_type=f32).astype(bf16)
            for g in range(4):
                k_ref[g, lo:hi, :] = kk[:, g * 128:(g + 1) * 128]
            qT = lax.dot_general(wqT, h, _NT, preferred_element_type=f32)
            qT_ref[:, lo:hi] = (qT * QSCALE).astype(bf16)
            vT = lax.dot_general(wvT, h, _NT, preferred_element_type=f32)
            vT_ref[:, lo:hi] = vT.astype(bf16)

    q0 = pl.multiple_of(step * TQ, TQ)
    nsteps = pl.num_programs(0)
    qn = pl.multiple_of(jnp.minimum(step + 1, nsteps - 1) * TQ, TQ)

    @pl.when(step == 0)
    def _():
        w_ref[0, 0:16, :] = qT_ref[0:16, 0:TQ]
    for h in range(1, H):
        j = h % 8
        w_ref[h, j * 16:(j + 1) * 16, :] = qT_ref[h * 16:(h + 1) * 16, pl.ds(q0, TQ)]
    w_ref[H, 0:16, :] = qT_ref[0:16, pl.ds(qn, TQ)]

    def fused(h1, h2):
        if h1 is not None:
            g = (h1 // 8) % 4
            w = w_ref[h1]
            m8 = None
        if h2 is not None:
            m = jnp.broadcast_to(jnp.max(m_ref[...], axis=0, keepdims=True), (8, TQ))
            l8s = []
            acc = None
        for c in range(NK):
            if h2 is not None:
                mm = m
                if c >= LAG:
                    mm = jnp.where(l8s[c - LAG] < 0.0, 0.0, m)
                p = jnp.exp2(s_ref[c * TK:(c + 1) * TK, :].reshape(TK // 8, 8, TQ) - mm[None])
                lc = jnp.sum(p, axis=0)
                l8s.append(lc if not l8s else l8s[-1] + lc)
                vh = vT_ref[pl.ds(pl.multiple_of(h2 * 16, 16), 16), c * TK:(c + 1) * TK]
                a = jnp.dot(vh, p.reshape(TK, TQ).astype(bf16), preferred_element_type=f32)
                acc = a if acc is None else acc + a
            if h1 is not None:
                sT = jnp.dot(k_ref[g, c * TK:(c + 1) * TK, :], w, preferred_element_type=f32)
                s_ref[c * TK:(c + 1) * TK, :] = sT
                mc = jnp.max(sT.reshape(TK // 8, 8, TQ), axis=0)
                m8 = mc if m8 is None else jnp.maximum(m8, mc)
        if h1 is not None:
            m_ref[...] = m8
        if h2 is not None:
            l = jnp.sum(l8s[-1], axis=0, keepdims=True)
            oT_ref[pl.ds(pl.multiple_of(h2 * 16, 16), 16), :] = acc / l

    @pl.when(step == 0)
    def _():
        fused(0, None)

    def body(h, carry):
        fused(h + 1, h)
        return carry

    lax.fori_loop(0, H - 1, body, 0)

    @pl.when(step < nsteps - 1)
    def _():
        fused(H, H - 1)

    @pl.when(step == nsteps - 1)
    def _():
        fused(None, H - 1)

    @pl.when(step == 0)
    def _():
        cp_wmod_b().wait()
        mod_ref[:, 2 * D:6 * D] = jnp.dot(silu_c(), wmod_ref[:, 2 * D:6 * D], preferred_element_type=f32)
        cp_wo().wait()
        cp_w1().wait()
        cp_w2().wait()

    ga = mod_ref[0:1, 2 * D:3 * D]
    sb = mod_ref[0:1, 3 * D:4 * D]
    cb = mod_ref[0:1, 4 * D:5 * D]
    gb = mod_ref[0:1, 5 * D:6 * D]
    for lo in range(0, TQ, FB):
        o = oT_ref[:, lo:lo + FB].T.astype(bf16)
        attn = jnp.dot(o, wo_ref[...], preferred_element_type=f32)
        x1 = x_ref[pl.ds(pl.multiple_of(q0 + lo, FB), FB), :].astype(f32) + ga * attn
        h2 = (_ln(x1) * (1.0 + cb) + sb).astype(bf16)
        u = jnp.dot(h2, w1_ref[...], preferred_element_type=f32) + b1_ref[...].astype(f32).reshape(1, F)
        r = jnp.maximum(u, 0.0)
        hh = (r * r).astype(bf16)
        y = jnp.dot(hh, w2_ref[...], preferred_element_type=f32) + b2_ref[...].astype(f32).reshape(1, D)
        out_ref[lo:lo + FB, :] = (x1 + gb * y).astype(out_ref.dtype)


@jax.jit
def pallas_adaLN_cond__mha_block__dense_activation_squared_relu__prompt_kernel(
    A_x: jax.Array,
    A_wqkv: jax.Array,
    A_wo: jax.Array,
    B_x: jax.Array,
    B_w1: jax.Array,
    B_b1: jax.Array,
    B_w2: jax.Array,
    B_b2: jax.Array,
    c: jax.Array,
    w_mod: jax.Array,
):
    del B_x
    x2 = A_x.reshape(S, D)
    b1 = B_b1
    b2 = B_b2

    def full(shape):
        return pl.BlockSpec(shape, lambda i: (0,) * len(shape))

    hbm = pl.BlockSpec(memory_space=pl.ANY)
    bf16 = jnp.bfloat16

    out = pl.pallas_call(
        _kernel,
        grid=(S // TQ,),
        in_specs=[hbm, hbm, hbm, hbm, full((F,)), hbm, full((D,)), full((1, D)), hbm],
        out_specs=pl.BlockSpec((TQ, D), lambda i: (i, 0)),
        out_shape=jax.ShapeDtypeStruct((S, D), A_x.dtype),
        scratch_shapes=[
            pltpu.VMEM((S, D), bf16),
            pltpu.VMEM((D, 3 * D), bf16),
            pltpu.VMEM((D, D), bf16),
            pltpu.VMEM((D, F), bf16),
            pltpu.VMEM((F, D), bf16),
            pltpu.VMEM((D, 6 * D), bf16),
            pltpu.SemaphoreType.DMA((10,)),
            pltpu.VMEM((8, 6 * D), jnp.float32),
            pltpu.VMEM((4, S, 128), bf16),
            pltpu.VMEM((D, S), bf16),
            pltpu.VMEM((D, S), bf16),
            pltpu.VMEM((H + 1, 128, TQ), bf16),
            pltpu.VMEM((S, TQ), jnp.float32),
            pltpu.VMEM((8, TQ), jnp.float32),
            pltpu.VMEM((D, TQ), jnp.float32),
        ],
        compiler_params=pltpu.CompilerParams(
            dimension_semantics=("arbitrary",),
            vmem_limit_bytes=100 * 1024 * 1024,
        ),
    )(x2, A_wqkv, A_wo, B_w1, b1, B_w2, b2, c, w_mod)
    return out.reshape(A_x.shape)
```

```python
import functools
import math

import jax
import jax.numpy as jnp
from jax import lax
import jax.experimental.pallas as pl
import jax.experimental.pallas.tpu as pltpu

S = 2048
D = 512
H = 32
DH = 16
F = 1792
TQ = 512
TK = 128
NK = S // TK
XB = (0, 256, 2048)
RBS = (0, 256, 384, 768, 1280, 2048)
LAG = 3
NB = 4
FB = 512
EPS = 1e-5
QSCALE = (DH ** -0.5) * math.log2(math.e)

_NT = (((1,), (1,)), ((), ()))


def _ln(x):
    mu = jnp.mean(x, axis=-1, keepdims=True)
    xc = x - mu
    var = jnp.mean(xc * xc, axis=-1, keepdims=True)
    return xc * lax.rsqrt(var + EPS)


def _kernel(x_hbm, wqkv_hbm, wo_hbm, w1_hbm, b1_ref, w2_hbm, b2_ref, c_ref, wmod_hbm,
            out_ref,
            x_ref, wqkv_ref, wo_ref, w1_ref, w2_ref, wmod_ref, sems,
            mod_ref, k_ref, qT_ref, vT_ref, w_ref, oT_ref, *sm_refs):
    s_refs, m_refs = sm_refs[:NB], sm_refs[NB:]
    step = pl.program_id(0)
    f32 = jnp.float32
    bf16 = jnp.bfloat16

    def cp_wmod_a():
        return pltpu.make_async_copy(wmod_hbm.at[:, 0:2 * D], wmod_ref.at[:, 0:2 * D], sems.at[0])

    def cp_x(r):
        lo, hi = XB[r], XB[r + 1]
        return pltpu.make_async_copy(x_hbm.at[lo:hi, :], x_ref.at[lo:hi, :], sems.at[1 + r])

    def cp_wqkv():
        return pltpu.make_async_copy(wqkv_hbm, wqkv_ref, sems.at[5])

    def cp_wmod_b():
        return pltpu.make_async_copy(wmod_hbm.at[:, 2 * D:6 * D], wmod_ref.at[:, 2 * D:6 * D], sems.at[6])

    def cp_wo():
        return pltpu.make_async_copy(wo_hbm, wo_ref, sems.at[7])

    def cp_w1():
        return pltpu.make_async_copy(w1_hbm, w1_ref, sems.at[8])

    def cp_w2():
        return pltpu.make_async_copy(w2_hbm, w2_ref, sems.at[9])

    def silu_c():
        cc = jnp.broadcast_to(c_ref[...].astype(f32), (8, D))
        return (cc * jax.nn.sigmoid(cc)).astype(bf16)

    @pl.when(step == 0)
    def _():
        cp_wmod_a().start()
        cp_x(0).start()
        cp_wqkv().start()
        cp_x(1).start()

        w_ref[...] = jnp.zeros_like(w_ref)
        cp_wmod_a().wait()
        mod_ref[:, 0:2 * D] = jnp.dot(silu_c(), wmod_ref[:, 0:2 * D], preferred_element_type=f32)
        sa = mod_ref[0:1, 0 * D:1 * D]
        ca = mod_ref[0:1, 1 * D:2 * D]
        cp_wqkv().wait()
        cp_x(0).wait()
        cp_wmod_b().start()
        cp_wo().start()
        cp_w1().start()
        cp_w2().start()
        wqT = wqkv_ref[:, 0:D].T
        wvT = wqkv_ref[:, 2 * D:3 * D].T
        for r in range(len(RBS) - 1):
            lo, hi = RBS[r], RBS[r + 1]
            if lo == XB[1]:
                cp_x(1).wait()
            xr = x_ref[lo:hi, :].astype(f32)
            h = (_ln(xr) * (1.0 + ca) + sa).astype(bf16)
            kk = jnp.dot(h, wqkv_ref[:, D:2 * D], preferred_element_type=f32).astype(bf16)
            for g in range(4):
                k_ref[g, lo:hi, :] = kk[:, g * 128:(g + 1) * 128]
            qT = lax.dot_general(wqT, h, _NT, preferred_element_type=f32)
            qT_ref[:, lo:hi] = (qT * QSCALE).astype(bf16)
            vT = lax.dot_general(wvT, h, _NT, preferred_element_type=f32)
            vT_ref[:, lo:hi] = vT.astype(bf16)

    q0 = pl.multiple_of(step * TQ, TQ)
    nsteps = pl.num_programs(0)
    qn = pl.multiple_of(jnp.minimum(step + 1, nsteps - 1) * TQ, TQ)

    @pl.when(step == 0)
    def _():
        for h in range(NB):
            w_ref[h, h * 16:(h + 1) * 16, :] = qT_ref[h * 16:(h + 1) * 16, 0:TQ]
    for h in range(NB, H):
        j = h % 8
        w_ref[h, j * 16:(j + 1) * 16, :] = qT_ref[h * 16:(h + 1) * 16, pl.ds(q0, TQ)]
    for h in range(NB):
        w_ref[H + h, h * 16:(h + 1) * 16, :] = qT_ref[h * 16:(h + 1) * 16, pl.ds(qn, TQ)]

    def fused(h1, h2, s_ref, m_ref):
        if h1 is not None:
            g = (h1 // 8) % 4
            w = w_ref[h1]
            m8 = None
        if h2 is not None:
            m = jnp.broadcast_to(jnp.max(m_ref[...], axis=0, keepdims=True), (8, TQ))
            l8s = []
            acc = None
        for c in range(NK):
            if h2 is not None:
                mm = m
                if c >= LAG:
                    mm = jnp.where(l8s[c - LAG] < 0.0, 0.0, m)
                p = jnp.exp2(s_ref[c * TK:(c + 1) * TK, :].reshape(TK // 8, 8, TQ) - mm[None])
                lc = jnp.sum(p, axis=0)
                l8s.append(lc if not l8s else l8s[-1] + lc)
                vh = vT_ref[pl.ds(pl.multiple_of(h2 * 16, 16), 16), c * TK:(c + 1) * TK]
                a = jnp.dot(vh, p.reshape(TK, TQ).astype(bf16), preferred_element_type=f32)
                acc = a if acc is None else acc + a
            if h1 is not None:
                sT = jnp.dot(k_ref[g, c * TK:(c + 1) * TK, :], w, preferred_element_type=f32)
                s_ref[c * TK:(c + 1) * TK, :] = sT
                mc = jnp.max(sT.reshape(TK // 8, 8, TQ), axis=0)
                m8 = mc if m8 is None else jnp.maximum(m8, mc)
        if h1 is not None:
            m_ref[...] = m8
        if h2 is not None:
            l = jnp.sum(l8s[-1], axis=0, keepdims=True)
            oT_ref[pl.ds(pl.multiple_of(h2 * 16, 16), 16), :] = acc / l

    @pl.when(step == 0)
    def _():
        for u in range(NB):
            fused(u, None, s_refs[u], m_refs[u])

    def body(i, carry):
        for u in range(NB):
            fused(i * NB + u + NB, i * NB + u, s_refs[u], m_refs[u])
        return carry

    lax.fori_loop(0, jnp.where(step == nsteps - 1, H // NB - 1, H // NB), body, 0)

    @pl.when(step == nsteps - 1)
    def _():
        for u in range(NB):
            fused(None, H - NB + u, s_refs[u], m_refs[u])

    @pl.when(step == 0)
    def _():
        cp_wmod_b().wait()
        mod_ref[:, 2 * D:6 * D] = jnp.dot(silu_c(), wmod_ref[:, 2 * D:6 * D], preferred_element_type=f32)
        cp_wo().wait()
        cp_w1().wait()
        cp_w2().wait()

    ga = mod_ref[0:1, 2 * D:3 * D]
    sb = mod_ref[0:1, 3 * D:4 * D]
    cb = mod_ref[0:1, 4 * D:5 * D]
    gb = mod_ref[0:1, 5 * D:6 * D]
    for lo in range(0, TQ, FB):
        o = oT_ref[:, lo:lo + FB].T.astype(bf16)
        attn = jnp.dot(o, wo_ref[...], preferred_element_type=f32)
        x1 = x_ref[pl.ds(pl.multiple_of(q0 + lo, FB), FB), :].astype(f32) + ga * attn
        h2 = (_ln(x1) * (1.0 + cb) + sb).astype(bf16)
        u = jnp.dot(h2, w1_ref[...], preferred_element_type=f32) + b1_ref[...].astype(f32).reshape(1, F)
        r = jnp.maximum(u, 0.0)
        hh = (r * r).astype(bf16)
        y = jnp.dot(hh, w2_ref[...], preferred_element_type=f32) + b2_ref[...].astype(f32).reshape(1, D)
        out_ref[lo:lo + FB, :] = (x1 + gb * y).astype(out_ref.dtype)


@jax.jit
def pallas_adaLN_cond__mha_block__dense_activation_squared_relu__prompt_kernel(
    A_x: jax.Array,
    A_wqkv: jax.Array,
    A_wo: jax.Array,
    B_x: jax.Array,
    B_w1: jax.Array,
    B_b1: jax.Array,
    B_w2: jax.Array,
    B_b2: jax.Array,
    c: jax.Array,
    w_mod: jax.Array,
):
    del B_x
    x2 = A_x.reshape(S, D)
    b1 = B_b1
    b2 = B_b2

    def full(shape):
        return pl.BlockSpec(shape, lambda i: (0,) * len(shape))

    hbm = pl.BlockSpec(memory_space=pl.ANY)
    bf16 = jnp.bfloat16

    out = pl.pallas_call(
        _kernel,
        grid=(S // TQ,),
        in_specs=[hbm, hbm, hbm, hbm, full((F,)), hbm, full((D,)), full((1, D)), hbm],
        out_specs=pl.BlockSpec((TQ, D), lambda i: (i, 0)),
        out_shape=jax.ShapeDtypeStruct((S, D), A_x.dtype),
        scratch_shapes=[
            pltpu.VMEM((S, D), bf16),
            pltpu.VMEM((D, 3 * D), bf16),
            pltpu.VMEM((D, D), bf16),
            pltpu.VMEM((D, F), bf16),
            pltpu.VMEM((F, D), bf16),
            pltpu.VMEM((D, 6 * D), bf16),
            pltpu.SemaphoreType.DMA((10,)),
            pltpu.VMEM((8, 6 * D), jnp.float32),
            pltpu.VMEM((4, S, 128), bf16),
            pltpu.VMEM((D, S), bf16),
            pltpu.VMEM((D, S), bf16),
            pltpu.VMEM((H + NB, 128, TQ), bf16),
            pltpu.VMEM((D, TQ), jnp.float32),
        ] + [pltpu.VMEM((S, TQ), jnp.float32)] * NB
          + [pltpu.VMEM((8, TQ), jnp.float32)] * NB,
        compiler_params=pltpu.CompilerParams(
            dimension_semantics=("arbitrary",),
            vmem_limit_bytes=100 * 1024 * 1024,
        ),
    )(x2, A_wqkv, A_wo, B_w1, b1, B_w2, b2, c, w_mod)
    return out.reshape(A_x.shape)
```

```python
import math

import jax
import jax.numpy as jnp
from jax import lax
import jax.experimental.pallas as pl
import jax.experimental.pallas.tpu as pltpu

S = 2048
D = 512
H = 32
DH = 16
F = 1792
TQ = 512
TK = 128
NK = S // TK
XB = (0, 256, 2048)
RBS = (0, 256, 384, 768, 1280, 2048)
LAG = 3
NB = 4
FB = 512
EPS = 1e-5
QSCALE = (DH ** -0.5) * math.log2(math.e)

_NT = (((1,), (1,)), ((), ()))


def _ln(x):
    mu = jnp.mean(x, axis=-1, keepdims=True)
    xc = x - mu
    var = jnp.mean(xc * xc, axis=-1, keepdims=True)
    return xc * lax.rsqrt(var + EPS)


def _kernel(x_hbm, wqkv_hbm, wo_hbm, w1_hbm, b1_ref, w2_hbm, b2_ref, c_ref, wmod_hbm,
            out_ref,
            x_ref, wqkv_ref, wo_ref, w1_ref, w2_ref, wmod_ref, sems,
            mod_ref, k_ref, qT_ref, vT_ref, w_ref, oT_ref, *sm_refs):
    s_refs, m_refs = sm_refs[:NB], sm_refs[NB:]
    step = pl.program_id(0)
    f32 = jnp.float32
    bf16 = jnp.bfloat16

    def cp_wmod_a():
        return pltpu.make_async_copy(wmod_hbm.at[:, 0:2 * D], wmod_ref.at[:, 0:2 * D], sems.at[0])

    def cp_x(r):
        lo, hi = XB[r], XB[r + 1]
        return pltpu.make_async_copy(x_hbm.at[lo:hi, :], x_ref.at[lo:hi, :], sems.at[1 + r])

    def cp_wqkv():
        return pltpu.make_async_copy(wqkv_hbm, wqkv_ref, sems.at[5])

    def cp_wmod_b():
        return pltpu.make_async_copy(wmod_hbm.at[:, 2 * D:6 * D], wmod_ref.at[:, 2 * D:6 * D], sems.at[6])

    def cp_wo():
        return pltpu.make_async_copy(wo_hbm, wo_ref, sems.at[7])

    def cp_w1():
        return pltpu.make_async_copy(w1_hbm, w1_ref, sems.at[8])

    def cp_w2():
        return pltpu.make_async_copy(w2_hbm, w2_ref, sems.at[9])

    def silu_c():
        cc = jnp.broadcast_to(c_ref[...].astype(f32), (8, D))
        return (cc * jax.nn.sigmoid(cc)).astype(bf16)

    @pl.when(step == 0)
    def _():
        cp_wmod_a().start()
        cp_x(0).start()
        cp_wqkv().start()
        cp_x(1).start()

        w_ref[...] = jnp.zeros_like(w_ref)
        cp_wmod_a().wait()
        mod_ref[:, 0:2 * D] = jnp.dot(silu_c(), wmod_ref[:, 0:2 * D], preferred_element_type=f32)
        sa = mod_ref[0:1, 0 * D:1 * D]
        ca = mod_ref[0:1, 1 * D:2 * D]
        cp_wqkv().wait()
        cp_x(0).wait()
        cp_wmod_b().start()
        cp_wo().start()
        cp_w1().start()
        cp_w2().start()
        wqT = wqkv_ref[:, 0:D].T
        wvT = wqkv_ref[:, 2 * D:3 * D].T
        for r in range(len(RBS) - 1):
            lo, hi = RBS[r], RBS[r + 1]
            if lo == XB[1]:
                cp_x(1).wait()
            xr = x_ref[lo:hi, :].astype(f32)
            h = (_ln(xr) * (1.0 + ca) + sa).astype(bf16)
            kk = jnp.dot(h, wqkv_ref[:, D:2 * D], preferred_element_type=f32).astype(bf16)
            for g in range(4):
                k_ref[g, lo:hi, :] = kk[:, g * 128:(g + 1) * 128]
            qT = lax.dot_general(wqT, h, _NT, preferred_element_type=f32)
            qT_ref[:, lo:hi] = (qT * QSCALE).astype(bf16)
            vT = lax.dot_general(wvT, h, _NT, preferred_element_type=f32)
            vT_ref[:, lo:hi] = vT.astype(bf16)

    q0 = pl.multiple_of(step * TQ, TQ)
    nsteps = pl.num_programs(0)
    qn = pl.multiple_of(jnp.minimum(step + 1, nsteps - 1) * TQ, TQ)

    @pl.when(step == 0)
    def _():
        for h in range(NB):
            w_ref[h, h * 16:(h + 1) * 16, :] = qT_ref[h * 16:(h + 1) * 16, 0:TQ]
    for h in range(NB, H):
        j = h % 8
        w_ref[h, j * 16:(j + 1) * 16, :] = qT_ref[h * 16:(h + 1) * 16, pl.ds(q0, TQ)]
    for h in range(NB):
        w_ref[H + h, h * 16:(h + 1) * 16, :] = qT_ref[h * 16:(h + 1) * 16, pl.ds(qn, TQ)]

    def fused(h1, h2, s_ref, m_ref):
        if h1 is not None:
            g = (h1 // 8) % 4
            w = w_ref[h1]
            m8 = None
        if h2 is not None:
            m = jnp.broadcast_to(jnp.max(m_ref[...], axis=0, keepdims=True), (8, TQ))
            l8s = []
            acc = None
        for c in range(NK):
            if h2 is not None:
                mm = m
                if c >= LAG:
                    mm = jnp.where(l8s[c - LAG] < 0.0, 0.0, m)
                p = jnp.exp2(s_ref[c * TK:(c + 1) * TK, :].reshape(TK // 8, 8, TQ) - mm[None])
                lc = jnp.sum(p, axis=0)
                l8s.append(lc if not l8s else l8s[-1] + lc)
                vh = vT_ref[pl.ds(pl.multiple_of(h2 * 16, 16), 16), c * TK:(c + 1) * TK]
                a = jnp.dot(vh, p.reshape(TK, TQ).astype(bf16), preferred_element_type=f32)
                acc = a if acc is None else acc + a
            if h1 is not None:
                sT = jnp.dot(k_ref[g, c * TK:(c + 1) * TK, :], w, preferred_element_type=f32)
                s_ref[c * TK:(c + 1) * TK, :] = sT
                mc = jnp.max(sT.reshape(TK // 8, 8, TQ), axis=0)
                m8 = mc if m8 is None else jnp.maximum(m8, mc)
        if h1 is not None:
            m_ref[...] = m8
        if h2 is not None:
            l = jnp.sum(l8s[-1], axis=0, keepdims=True)
            oT_ref[pl.ds(pl.multiple_of(h2 * 16, 16), 16), :] = acc / l

    @pl.when(step == 0)
    def _():
        for u in range(NB):
            fused(u, None, s_refs[u], m_refs[u])

    def body(i, carry):
        for u in range(NB):
            fused(i * NB + u + NB, i * NB + u, s_refs[u], m_refs[u])
        return carry

    lax.fori_loop(0, jnp.where(step == nsteps - 1, H // NB - 1, H // NB), body, 0)

    @pl.when(step == nsteps - 1)
    def _():
        for u in range(NB):
            fused(None, H - NB + u, s_refs[u], m_refs[u])

    @pl.when(step == 0)
    def _():
        cp_wmod_b().wait()
        mod_ref[:, 2 * D:6 * D] = jnp.dot(silu_c(), wmod_ref[:, 2 * D:6 * D], preferred_element_type=f32)
        cp_wo().wait()
        cp_w1().wait()
        cp_w2().wait()

    ga = mod_ref[0:1, 2 * D:3 * D]
    sb = mod_ref[0:1, 3 * D:4 * D]
    cb = mod_ref[0:1, 4 * D:5 * D]
    gb = mod_ref[0:1, 5 * D:6 * D]
    for lo in range(0, TQ, FB):
        o = oT_ref[:, lo:lo + FB].T.astype(bf16)
        attn = jnp.dot(o, wo_ref[...], preferred_element_type=f32)
        x1 = x_ref[pl.ds(pl.multiple_of(q0 + lo, FB), FB), :].astype(f32) + ga * attn
        h2 = (_ln(x1) * (1.0 + cb) + sb).astype(bf16)
        u = jnp.dot(h2, w1_ref[...], preferred_element_type=f32) + b1_ref[...].astype(f32).reshape(1, F)
        r = jnp.maximum(u, 0.0)
        hh = (r * r).astype(bf16)
        y = jnp.dot(hh, w2_ref[...], preferred_element_type=f32) + b2_ref[...].astype(f32).reshape(1, D)
        out_ref[lo:lo + FB, :] = (x1 + gb * y).astype(out_ref.dtype)


@jax.jit
def pallas_adaLN_cond__mha_block__dense_activation_squared_relu__prompt_kernel(
    A_x: jax.Array,
    A_wqkv: jax.Array,
    A_wo: jax.Array,
    B_x: jax.Array,
    B_w1: jax.Array,
    B_b1: jax.Array,
    B_w2: jax.Array,
    B_b2: jax.Array,
    c: jax.Array,
    w_mod: jax.Array,
):
    del B_x
    x2 = A_x.reshape(S, D)

    def full(shape):
        return pl.BlockSpec(shape, lambda i: (0,) * len(shape))

    hbm = pl.BlockSpec(memory_space=pl.ANY)
    bf16 = jnp.bfloat16

    out = pl.pallas_call(
        _kernel,
        grid=(S // TQ,),
        in_specs=[hbm, hbm, hbm, hbm, full((F,)), hbm, full((D,)), full((1, D)), hbm],
        out_specs=pl.BlockSpec((TQ, D), lambda i: (i, 0)),
        out_shape=jax.ShapeDtypeStruct((S, D), A_x.dtype),
        scratch_shapes=[
            pltpu.VMEM((S, D), bf16),
            pltpu.VMEM((D, 3 * D), bf16),
            pltpu.VMEM((D, D), bf16),
            pltpu.VMEM((D, F), bf16),
            pltpu.VMEM((F, D), bf16),
            pltpu.VMEM((D, 6 * D), bf16),
            pltpu.SemaphoreType.DMA((10,)),
            pltpu.VMEM((8, 6 * D), jnp.float32),
            pltpu.VMEM((4, S, 128), bf16),
            pltpu.VMEM((D, S), bf16),
            pltpu.VMEM((D, S), bf16),
            pltpu.VMEM((H + NB, 128, TQ), bf16),
            pltpu.VMEM((D, TQ), jnp.float32),
        ] + [pltpu.VMEM((S, TQ), jnp.float32)] * NB
          + [pltpu.VMEM((8, TQ), jnp.float32)] * NB,
        compiler_params=pltpu.CompilerParams(
            dimension_semantics=("arbitrary",),
            vmem_limit_bytes=100 * 1024 * 1024,
        ),
    )(x2, A_wqkv, A_wo, B_w1, B_b1, B_w2, B_b2, c, w_mod)
    return out.reshape(A_x.shape)
```
